```python
import os as _os
_os.environ.setdefault("JAX_PLATFORMS", "cpu")
import jax
import jax.numpy as jnp

def _softmax(x, axis=-1):
    return jax.nn.softmax(x, axis=axis)
def _gelu(x):
    return jax.nn.gelu(x, approximate=True)
def _silu(x):
    return jax.nn.silu(x)
def _sigmoid(x):
    return jax.nn.sigmoid(x)
def _layernorm(x, axis=-1, eps=1e-5):
    m = jnp.mean(x, axis=axis, keepdims=True)
    v = jnp.var(x, axis=axis, keepdims=True)
    return (x - m) / jnp.sqrt(v + eps)
def _scatter_add(tgt, idx, src, axis=0):
    return tgt.at[idx].add(src)
def _segment_sum(src, seg, n):
    return jax.ops.segment_sum(src, seg, n)
class _Rng:
    def __init__(self, key):
        self._k = key
    def _next(self):
        self._k, sub = jax.random.split(self._k)
        return sub
    def normal(self, shape):
        return jax.random.normal(self._next(), shape, dtype=jnp.bfloat16)
    def randint(self, lo, hi, shape):
        return jax.random.randint(self._next(), shape, lo, hi, dtype=jnp.int32)
    def uniform(self, shape, lo=0.0, hi=1.0):
        return jax.random.uniform(self._next(), shape, jnp.bfloat16, lo, hi)
    def permutation(self, n):
        return jax.random.permutation(self._next(), n)


kernel_name = 'gated_mix__ssm_conv_s5__geglu_ffn__prompt'

def setup_inputs():
    _rng = _Rng(jax.random.key(int.from_bytes(__import__("os").urandom(4), "little")))
    _w = (lambda a: (lambda t: t.astype(jnp.bfloat16) if jnp.issubdtype(t.dtype, jnp.floating) else t)(jnp.asarray(a)))
    def _A_setup():
        B, S, D = 1, 2048, 512
        P = D
        Lambda_re = -0.5 * jnp.exp((lambda *s: _rng.normal(s) * 0.4)(P))
        Lambda_im = (lambda *s: _rng.normal(s) * 0.4)(P) * 1.0
        B_re = (lambda *s: _rng.normal(s) * 0.4)(P, D) * (D ** -0.5)
        B_im = (lambda *s: _rng.normal(s) * 0.4)(P, D) * (D ** -0.5)
        C_re = (lambda *s: _rng.normal(s) * 0.4)(D, P) * (P ** -0.5)
        C_im = (lambda *s: _rng.normal(s) * 0.4)(D, P) * (P ** -0.5)
        log_dt = (lambda *s: _rng.normal(s) * 0.4)(P) * 0.3 - 2.0
        Dskip = (lambda *s: _rng.normal(s) * 0.4)(D)
        return {
            "x": _w((lambda *s: _rng.normal(s) * 0.05)(B, S, D)),
            "Lambda_re": _w(Lambda_re),
            "Lambda_im": _w(Lambda_im),
            "B_re": _w(B_re),
            "B_im": _w(B_im),
            "C_re": _w(C_re),
            "C_im": _w(C_im),
            "log_dt": _w(log_dt),
            "Dskip": _w(Dskip),
        }
    _A_in = _A_setup()

    def _B_setup():
        B, S, D, F = 1, 2048, 512, 1376
        return {
            "x": _w((lambda *s: _rng.normal(s) * 0.05)(B, S, D)),
            "w_gate": _w((lambda *s: _rng.normal(s) * 0.1)(D, F)),
            "w_up": _w((lambda *s: _rng.normal(s) * 0.1)(D, F)),
            "w_down": _w((lambda *s: _rng.normal(s) * 0.1)(F, D)),
        }
    _B_in = _B_setup()

    return {
        "A_x": _A_in["x"],
        "A_Lambda_re": _A_in["Lambda_re"],
        "A_Lambda_im": _A_in["Lambda_im"],
        "A_B_re": _A_in["B_re"],
        "A_B_im": _A_in["B_im"],
        "A_C_re": _A_in["C_re"],
        "A_C_im": _A_in["C_im"],
        "A_log_dt": _A_in["log_dt"],
        "A_Dskip": _A_in["Dskip"],
        "B_x": _B_in["x"],
        "B_w_gate": _B_in["w_gate"],
        "B_w_up": _B_in["w_up"],
        "B_w_down": _B_in["w_down"],
        "gate_w": _w((lambda *s: _rng.normal(s) * 0.05)(512) * 16.0),
    }

def reference(A_x, A_Lambda_re, A_Lambda_im, A_B_re, A_B_im, A_C_re, A_C_im, A_log_dt, A_Dskip, B_x, B_w_gate, B_w_up, B_w_down, gate_w):
    def _A_ref(x, Lambda_re, Lambda_im, B_re, B_im, C_re, C_im, log_dt, Dskip):
        Bsz, L, H = x.shape
        Lam = Lambda_re + 1j * Lambda_im
        Bmat = B_re + 1j * B_im
        Cmat = C_re + 1j * C_im
        dt = jnp.exp(log_dt)
        Lam_bar = jnp.exp(dt * Lam)
        B_bar = ((Lam_bar - 1.0) / Lam)[:, None] * Bmat
        Bu = jnp.einsum("bld,pd->blp", x + 0j, B_bar)
        h = jnp.zeros_like(Bu[:, 0, :])
        hs = []
        for t in range(L):
            h = Lam_bar[None, :] * h + Bu[:, t, :]
            hs.append(h)
        hseq = jnp.stack(hs, 1)
        y = 2.0 * jnp.einsum("blp,dp->bld", hseq, Cmat).real + x * Dskip[None, None, :]
        return y

    def _B_ref(x, w_gate, w_up, w_down):
        return (_gelu(x @ w_gate) * (x @ w_up)) @ w_down

    x = A_x
    g = _sigmoid((x * gate_w).sum(-1, keepdims=True))
    a = _A_ref(x, A_Lambda_re, A_Lambda_im, A_B_re, A_B_im, A_C_re, A_C_im, A_log_dt, A_Dskip)
    b = _B_ref(x, B_w_gate, B_w_up, B_w_down)
    return g * a + (1 - g) * b
```

```python
import functools

import jax
import jax.numpy as jnp
from jax import lax
import jax.experimental.pallas as pl
import jax.experimental.pallas.tpu as pltpu

F32 = jnp.float32
BF16 = jnp.bfloat16

TM = 256
NSEG = 8


def _cmul(ar, ai, br, bi):
    return ar * br - ai * bi, ar * bi + ai * br


def _kernel(x_ref, lre_ref, lim_ref, bre_ref, bim_ref, cre_ref, cim_ref, ldt_ref,
            dsk_ref, wg_ref, wu_ref, wd_ref, gw_ref,
            o_ref,
            lam_ref, wc_ref, z_ref, carry_ref, *, tm):
    P = lre_ref.shape[1]
    seg = tm // NSEG
    step = pl.program_id(0)

    @pl.when(step == 0)
    def _prep():
        lre = lre_ref[...].astype(F32)
        lim = lim_ref[...].astype(F32)
        dt = jnp.exp(ldt_ref[...].astype(F32)).astype(BF16).astype(F32)
        mag = jnp.exp(dt * lre)
        ang = dt * lim
        lbr = mag * jnp.cos(ang)
        lbi = mag * jnp.sin(ang)
        nr = lbr - 1.0
        ni = lbi
        den = lre * lre + lim * lim
        cr = (nr * lre + ni * lim) / den
        ci = (ni * lre - nr * lim) / den
        pr, pi_ = lbr, lbi
        n = 1
        while n < seg:
            pr, pi_ = _cmul(pr, pi_, pr, pi_)
            n *= 2
        lam_ref[0:1, :] = lbr
        lam_ref[1:2, :] = lbi
        lam_ref[2:3, :] = pr
        lam_ref[3:4, :] = pi_
        lam_ref[4:8, :] = jnp.zeros((4, P), F32)
        cre = cre_ref[...].astype(F32)
        cim = cim_ref[...].astype(F32)
        wc_ref[:, 0:P] = (2.0 * (cre * cr - cim * ci)).astype(BF16)
        wc_ref[:, P:2 * P] = (-2.0 * (cre * ci + cim * cr)).astype(BF16)
        carry_ref[...] = jnp.zeros(carry_ref.shape, F32)

    x = x_ref[...]
    nt = (((1,), (1,)), ((), ()))
    NC = P // 128
    zr = lax.dot_general(x, bre_ref[...], nt, preferred_element_type=F32)
    for c in range(NC):
        z_ref[c] = zr[:, c * 128:(c + 1) * 128]
    zi = lax.dot_general(x, bim_ref[...], nt, preferred_element_type=F32)
    for c in range(NC):
        z_ref[NC + c] = zi[:, c * 128:(c + 1) * 128]

    def load_z(k):
        zr_ = jnp.concatenate(
            [z_ref[c, pl.ds(k, NSEG, stride=seg), :] for c in range(NC)], axis=1)
        zi_ = jnp.concatenate(
            [z_ref[NC + c, pl.ds(k, NSEG, stride=seg), :] for c in range(NC)], axis=1)
        return zr_, zi_

    lbr = jnp.broadcast_to(lam_ref[0:1, :], (NSEG, P))
    lbi = jnp.broadcast_to(lam_ref[1:2, :], (NSEG, P))

    def body1(k, c):
        er, ei = c
        zr_, zi_ = load_z(k)
        er, ei = _cmul(lbr, lbi, er, ei)
        return er + zr_, ei + zi_

    z0 = jnp.zeros((NSEG, P), F32)
    er, ei = lax.fori_loop(0, seg, body1, (z0, z0), unroll=8)

    psr = lam_ref[2:3, :]
    psi = lam_ref[3:4, :]
    hr = carry_ref[0:1, :]
    hi = carry_ref[1:2, :]
    inits_r = []
    inits_i = []
    for j in range(NSEG):
        inits_r.append(hr)
        inits_i.append(hi)
        hr, hi = _cmul(psr, psi, hr, hi)
        hr = hr + er[j:j + 1, :]
        hi = hi + ei[j:j + 1, :]
    carry_ref[0:1, :] = hr
    carry_ref[1:2, :] = hi
    h0r = jnp.concatenate(inits_r, axis=0)
    h0i = jnp.concatenate(inits_i, axis=0)

    def body2(k, c):
        hr, hi = c
        zr_, zi_ = load_z(k)
        hr, hi = _cmul(lbr, lbi, hr, hi)
        hr = hr + zr_
        hi = hi + zi_
        for c in range(NC):
            z_ref[c, pl.ds(k, NSEG, stride=seg), :] = hr[:, c * 128:(c + 1) * 128]
            z_ref[NC + c, pl.ds(k, NSEG, stride=seg), :] = hi[:, c * 128:(c + 1) * 128]
        return hr, hi

    lax.fori_loop(0, seg, body2, (h0r, h0i), unroll=8)

    xf = x.astype(F32)
    h = jnp.concatenate([z_ref[c].astype(BF16) for c in range(2 * NC)], axis=1)
    a = lax.dot_general(h, wc_ref[...], nt, preferred_element_type=F32)
    a = a + xf * dsk_ref[...].astype(F32)

    gate = jnp.dot(x, wg_ref[...], preferred_element_type=F32)
    up = jnp.dot(x, wu_ref[...], preferred_element_type=F32)
    act = (jax.nn.gelu(gate, approximate=True) * up).astype(BF16)
    b = jnp.dot(act, wd_ref[...], preferred_element_type=F32)

    logit = jnp.sum(xf * gw_ref[...].astype(F32), axis=-1, keepdims=True)
    g = jax.nn.sigmoid(logit)
    o_ref[...] = b + g * (a - b)


@functools.partial(jax.jit, static_argnames=("tm",))
def _run(A_x, A_Lambda_re, A_Lambda_im, A_B_re, A_B_im, A_C_re, A_C_im, A_log_dt,
         A_Dskip, B_w_gate, B_w_up, B_w_down, gate_w, tm=TM):
    Bsz, S, D = A_x.shape
    P = A_Lambda_re.shape[0]
    Fd = B_w_gate.shape[1]
    x2 = A_x.reshape(Bsz * S, D)
    row = lambda v: v.reshape(1, -1)

    full = lambda shape: pl.BlockSpec(shape, lambda i: (0,) * len(shape))
    out = pl.pallas_call(
        functools.partial(_kernel, tm=tm),
        grid=(S // tm,),
        in_specs=[
            pl.BlockSpec((tm, D), lambda i: (i, 0)),
            full((1, P)), full((1, P)),
            full((P, D)), full((P, D)),
            full((D, P)), full((D, P)),
            full((1, P)), full((1, D)),
            full((D, Fd)), full((D, Fd)), full((Fd, D)),
            full((1, D)),
        ],
        out_specs=pl.BlockSpec((tm, D), lambda i: (i, 0)),
        out_shape=jax.ShapeDtypeStruct((Bsz * S, D), F32),
        scratch_shapes=[
            pltpu.VMEM((8, P), F32),
            pltpu.VMEM((D, 2 * P), BF16),
            pltpu.VMEM((2 * P // 128, tm, 128), F32),
            pltpu.VMEM((8, P), F32),
        ],
        compiler_params=pltpu.CompilerParams(
            dimension_semantics=("arbitrary",),
            vmem_limit_bytes=64 * 1024 * 1024,
        ),
    )(x2, row(A_Lambda_re), row(A_Lambda_im), A_B_re, A_B_im, A_C_re, A_C_im,
      row(A_log_dt), row(A_Dskip), B_w_gate, B_w_up, B_w_down, row(gate_w))
    return out.reshape(Bsz, S, D)


@jax.jit
def pallas_gated_mix__ssm_conv_s5__geglu_ffn__prompt_kernel(
    A_x: jax.Array,
    A_Lambda_re: jax.Array,
    A_Lambda_im: jax.Array,
    A_B_re: jax.Array,
    A_B_im: jax.Array,
    A_C_re: jax.Array,
    A_C_im: jax.Array,
    A_log_dt: jax.Array,
    A_Dskip: jax.Array,
    B_x: jax.Array,
    B_w_gate: jax.Array,
    B_w_up: jax.Array,
    B_w_down: jax.Array,
    gate_w: jax.Array,
):
    return _run(A_x, A_Lambda_re, A_Lambda_im, A_B_re, A_B_im, A_C_re, A_C_im,
                A_log_dt, A_Dskip, B_w_gate, B_w_up, B_w_down, gate_w)
```

```python
import functools

import jax
import jax.numpy as jnp
from jax import lax
import jax.experimental.pallas as pl
import jax.experimental.pallas.tpu as pltpu

F32 = jnp.float32
BF16 = jnp.bfloat16

TM = 256
NSEG = 8


def _cmul(ar, ai, br, bi):
    return ar * br - ai * bi, ar * bi + ai * br


def _kernel(x_ref, lre_ref, lim_ref, bre_ref, bim_ref, cre_ref, cim_ref, ldt_ref,
            dsk_ref, wg_ref, wu_ref, wd_ref, gw_ref,
            o_ref,
            lam_ref, wc_ref, z_ref, carry_ref, *, tm):
    P = lre_ref.shape[1]
    step = pl.program_id(0)

    @pl.when(step == 0)
    def _prep():
        lre = lre_ref[...].astype(F32)
        lim = lim_ref[...].astype(F32)
        dt = jnp.exp(ldt_ref[...].astype(F32)).astype(BF16).astype(F32)
        mag = jnp.exp(dt * lre)
        ang = dt * lim
        lbr = mag * jnp.cos(ang)
        lbi = mag * jnp.sin(ang)
        nr = lbr - 1.0
        ni = lbi
        den = lre * lre + lim * lim
        cr = (nr * lre + ni * lim) / den
        ci = (ni * lre - nr * lim) / den
        pows = [(lbr, lbi)]
        for _ in range(7):
            pows.append(_cmul(pows[-1][0], pows[-1][1], lbr, lbi))
        row = lax.broadcasted_iota(jnp.int32, (8, P), 0)
        for idx, d in enumerate((1, 2, 4)):
            lam_ref[2 * idx] = jnp.where(row >= d, jnp.broadcast_to(pows[d - 1][0], (8, P)), 0.0)
            lam_ref[2 * idx + 1] = jnp.where(row >= d, jnp.broadcast_to(pows[d - 1][1], (8, P)), 0.0)
        lam_ref[6] = jnp.concatenate([p_[0] for p_ in pows], axis=0)
        lam_ref[7] = jnp.concatenate([p_[1] for p_ in pows], axis=0)
        cre = cre_ref[...].astype(F32)
        cim = cim_ref[...].astype(F32)
        wc_ref[:, 0:P] = (2.0 * (cre * cr - cim * ci)).astype(BF16)
        wc_ref[:, P:2 * P] = (-2.0 * (cre * ci + cim * cr)).astype(BF16)
        carry_ref[...] = jnp.zeros(carry_ref.shape, F32)

    x = x_ref[...]
    nt = (((1,), (1,)), ((), ()))
    z_ref[:, 0:P] = lax.dot_general(x, bre_ref[...], nt, preferred_element_type=F32)
    z_ref[:, P:2 * P] = lax.dot_general(x, bim_ref[...], nt, preferred_element_type=F32)

    cr_ = carry_ref[0:1, :]
    ci_ = carry_ref[1:2, :]
    for n in range(tm // 8):
        tr = z_ref[n * 8:(n + 1) * 8, 0:P]
        ti = z_ref[n * 8:(n + 1) * 8, P:2 * P]
        for idx, d in enumerate((1, 2, 4)):
            sr = pltpu.roll(tr, d, 0)
            si = pltpu.roll(ti, d, 0)
            mr, mi = _cmul(lam_ref[2 * idx], lam_ref[2 * idx + 1], sr, si)
            tr = tr + mr
            ti = ti + mi
        mr, mi = _cmul(lam_ref[6], lam_ref[7],
                       jnp.broadcast_to(cr_, (8, P)), jnp.broadcast_to(ci_, (8, P)))
        tr = tr + mr
        ti = ti + mi
        z_ref[n * 8:(n + 1) * 8, 0:P] = tr
        z_ref[n * 8:(n + 1) * 8, P:2 * P] = ti
        cr_ = tr[7:8, :]
        ci_ = ti[7:8, :]
    carry_ref[0:1, :] = cr_
    carry_ref[1:2, :] = ci_

    gate = lax.dot_general(x, wg_ref[...], nt, preferred_element_type=F32)
    up = lax.dot_general(x, wu_ref[...], nt, preferred_element_type=F32)
    act = (jax.nn.gelu(gate, approximate=True) * up).astype(BF16)
    b = jnp.dot(act, wd_ref[...], preferred_element_type=F32)

    xf = x.astype(F32)
    h = z_ref[...].astype(BF16)
    a = lax.dot_general(h, wc_ref[...], nt, preferred_element_type=F32)
    a = a + xf * dsk_ref[...].astype(F32)

    logit = jnp.sum(xf * gw_ref[...].astype(F32), axis=-1, keepdims=True)
    g = jax.nn.sigmoid(logit)
    o_ref[...] = b + g * (a - b)


@functools.partial(jax.jit, static_argnames=("tm",))
def _run(A_x, A_Lambda_re, A_Lambda_im, A_B_re, A_B_im, A_C_re, A_C_im, A_log_dt,
         A_Dskip, B_w_gate, B_w_up, B_w_down, gate_w, tm=TM):
    Bsz, S, D = A_x.shape
    P = A_Lambda_re.shape[0]
    Fd = B_w_gate.shape[1]
    x2 = A_x.reshape(Bsz * S, D)
    row = lambda v: v.reshape(1, -1)

    full = lambda shape: pl.BlockSpec(shape, lambda i: (0,) * len(shape))
    out = pl.pallas_call(
        functools.partial(_kernel, tm=tm),
        grid=(S // tm,),
        in_specs=[
            pl.BlockSpec((tm, D), lambda i: (i, 0)),
            full((1, P)), full((1, P)),
            full((P, D)), full((P, D)),
            full((D, P)), full((D, P)),
            full((1, P)), full((1, D)),
            full((Fd, D)), full((Fd, D)), full((Fd, D)),
            full((1, D)),
        ],
        out_specs=pl.BlockSpec((tm, D), lambda i: (i, 0)),
        out_shape=jax.ShapeDtypeStruct((Bsz * S, D), F32),
        scratch_shapes=[
            pltpu.VMEM((8, 8, P), F32),
            pltpu.VMEM((D, 2 * P), BF16),
            pltpu.VMEM((tm, 2 * P), F32),
            pltpu.VMEM((8, P), F32),
        ],
        compiler_params=pltpu.CompilerParams(
            dimension_semantics=("arbitrary",),
            vmem_limit_bytes=64 * 1024 * 1024,
        ),
    )(x2, row(A_Lambda_re), row(A_Lambda_im), A_B_re, A_B_im, A_C_re, A_C_im,
      row(A_log_dt), row(A_Dskip), B_w_gate.T, B_w_up.T, B_w_down, row(gate_w))
    return out.reshape(Bsz, S, D)


@jax.jit
def pallas_gated_mix__ssm_conv_s5__geglu_ffn__prompt_kernel(
    A_x: jax.Array,
    A_Lambda_re: jax.Array,
    A_Lambda_im: jax.Array,
    A_B_re: jax.Array,
    A_B_im: jax.Array,
    A_C_re: jax.Array,
    A_C_im: jax.Array,
    A_log_dt: jax.Array,
    A_Dskip: jax.Array,
    B_x: jax.Array,
    B_w_gate: jax.Array,
    B_w_up: jax.Array,
    B_w_down: jax.Array,
    gate_w: jax.Array,
):
    return _run(A_x, A_Lambda_re, A_Lambda_im, A_B_re, A_B_im, A_C_re, A_C_im,
                A_log_dt, A_Dskip, B_w_gate, B_w_up, B_w_down, gate_w)
```

```python
import functools

import jax
import jax.numpy as jnp
from jax import lax
import jax.experimental.pallas as pl
import jax.experimental.pallas.tpu as pltpu

F32 = jnp.float32
BF16 = jnp.bfloat16

TM = 256
NSEG = 8


def _cmul(ar, ai, br, bi):
    return ar * br - ai * bi, ar * bi + ai * br


def _kernel(x_ref, lre_ref, lim_ref, ldt_ref, dsk_ref, gw_ref, bre_ref, bim_ref,
            cre_hbm, cim_hbm, wg_hbm, wu_hbm, wd_hbm,
            o_ref,
            lam_ref, wc_ref, z_ref, carry_ref,
            cre_ref, cim_ref, wg_ref, wu_ref, wd_ref, sems, *, tm):
    P = lre_ref.shape[1]
    step = pl.program_id(0)
    nt = (((1,), (1,)), ((), ()))

    copies = [
        pltpu.make_async_copy(wg_hbm, wg_ref, sems.at[0]),
        pltpu.make_async_copy(wu_hbm, wu_ref, sems.at[1]),
        pltpu.make_async_copy(wd_hbm, wd_ref, sems.at[2]),
        pltpu.make_async_copy(cre_hbm, cre_ref, sems.at[3]),
        pltpu.make_async_copy(cim_hbm, cim_ref, sems.at[4]),
    ]

    def ssm_coefs():
        lre = lre_ref[...].astype(F32)
        lim = lim_ref[...].astype(F32)
        dt = jnp.exp(ldt_ref[...].astype(F32)).astype(BF16).astype(F32)
        mag = jnp.exp(dt * lre)
        ang = dt * lim
        lbr = mag * jnp.cos(ang)
        lbi = mag * jnp.sin(ang)
        nr = lbr - 1.0
        ni = lbi
        den = lre * lre + lim * lim
        cr = (nr * lre + ni * lim) / den
        ci = (ni * lre - nr * lim) / den
        return lbr, lbi, cr, ci

    def prep_lam(lbr, lbi):
        pows = [(lbr, lbi)]
        for _ in range(7):
            pows.append(_cmul(pows[-1][0], pows[-1][1], lbr, lbi))
        row = lax.broadcasted_iota(jnp.int32, (8, P), 0)
        for idx, d in enumerate((1, 2, 4)):
            lam_ref[2 * idx] = jnp.where(row >= d, jnp.broadcast_to(pows[d - 1][0], (8, P)), 0.0)
            lam_ref[2 * idx + 1] = jnp.where(row >= d, jnp.broadcast_to(pows[d - 1][1], (8, P)), 0.0)
        lam_ref[6] = jnp.concatenate([p_[0] for p_ in pows], axis=0)
        lam_ref[7] = jnp.concatenate([p_[1] for p_ in pows], axis=0)
        carry_ref[...] = jnp.zeros(carry_ref.shape, F32)

    def prep_wc(cr, ci):
        cre = cre_ref[...].astype(F32)
        cim = cim_ref[...].astype(F32)
        wc_ref[:, 0:P] = (2.0 * (cre * cr - cim * ci)).astype(BF16)
        wc_ref[:, P:2 * P] = (-2.0 * (cre * ci + cim * cr)).astype(BF16)

    def body(first):
        if first:
            for c in copies:
                c.start()
            lbr, lbi, cr, ci = ssm_coefs()
            prep_lam(lbr, lbi)

        x = x_ref[...]
        z_ref[:, 0:P] = lax.dot_general(x, bre_ref[...], nt, preferred_element_type=F32)
        z_ref[:, P:2 * P] = lax.dot_general(x, bim_ref[...], nt, preferred_element_type=F32)

        cr_ = carry_ref[0:1, :]
        ci_ = carry_ref[1:2, :]
        for n in range(tm // 8):
            tr = z_ref[n * 8:(n + 1) * 8, 0:P]
            ti = z_ref[n * 8:(n + 1) * 8, P:2 * P]
            for idx, d in enumerate((1, 2, 4)):
                sr = pltpu.roll(tr, d, 0)
                si = pltpu.roll(ti, d, 0)
                mr, mi = _cmul(lam_ref[2 * idx], lam_ref[2 * idx + 1], sr, si)
                tr = tr + mr
                ti = ti + mi
            mr, mi = _cmul(lam_ref[6], lam_ref[7],
                           jnp.broadcast_to(cr_, (8, P)), jnp.broadcast_to(ci_, (8, P)))
            tr = tr + mr
            ti = ti + mi
            z_ref[n * 8:(n + 1) * 8, 0:P] = tr
            z_ref[n * 8:(n + 1) * 8, P:2 * P] = ti
            cr_ = tr[7:8, :]
            ci_ = ti[7:8, :]
        carry_ref[0:1, :] = cr_
        carry_ref[1:2, :] = ci_

        if first:
            copies[0].wait()
        gate = lax.dot_general(x, wg_ref[...], nt, preferred_element_type=F32)
        if first:
            copies[1].wait()
        up = lax.dot_general(x, wu_ref[...], nt, preferred_element_type=F32)
        act = (jax.nn.gelu(gate, approximate=True) * up).astype(BF16)
        if first:
            copies[2].wait()
        b = jnp.dot(act, wd_ref[...], preferred_element_type=F32)

        if first:
            copies[3].wait()
            copies[4].wait()
            prep_wc(cr, ci)
        xf = x.astype(F32)
        h = z_ref[...].astype(BF16)
        a = lax.dot_general(h, wc_ref[...], nt, preferred_element_type=F32)
        a = a + xf * dsk_ref[...].astype(F32)

        logit = jnp.sum(xf * gw_ref[...].astype(F32), axis=-1, keepdims=True)
        g = jax.nn.sigmoid(logit)
        o_ref[...] = b + g * (a - b)

    @pl.when(step == 0)
    def _():
        body(True)

    @pl.when(step != 0)
    def _():
        body(False)


@functools.partial(jax.jit, static_argnames=("tm",))
def _run(A_x, A_Lambda_re, A_Lambda_im, A_B_re, A_B_im, A_C_re, A_C_im, A_log_dt,
         A_Dskip, B_w_gate, B_w_up, B_w_down, gate_w, tm=TM):
    Bsz, S, D = A_x.shape
    P = A_Lambda_re.shape[0]
    Fd = B_w_gate.shape[1]
    x2 = A_x.reshape(Bsz * S, D)
    row = lambda v: v.reshape(1, -1)

    full = lambda shape: pl.BlockSpec(shape, lambda i: (0,) * len(shape))
    hbm = pl.BlockSpec(memory_space=pl.ANY)
    out = pl.pallas_call(
        functools.partial(_kernel, tm=tm),
        grid=(S // tm,),
        in_specs=[
            pl.BlockSpec((tm, D), lambda i: (i, 0)),
            full((1, P)), full((1, P)), full((1, P)), full((1, D)), full((1, D)),
            full((P, D)), full((P, D)),
            hbm, hbm, hbm, hbm, hbm,
        ],
        out_specs=pl.BlockSpec((tm, D), lambda i: (i, 0)),
        out_shape=jax.ShapeDtypeStruct((Bsz * S, D), F32),
        scratch_shapes=[
            pltpu.VMEM((8, 8, P), F32),
            pltpu.VMEM((D, 2 * P), BF16),
            pltpu.VMEM((tm, 2 * P), F32),
            pltpu.VMEM((8, P), F32),
            pltpu.VMEM((D, P), BF16),
            pltpu.VMEM((D, P), BF16),
            pltpu.VMEM((Fd, D), BF16),
            pltpu.VMEM((Fd, D), BF16),
            pltpu.VMEM((Fd, D), BF16),
            pltpu.SemaphoreType.DMA((5,)),
        ],
        compiler_params=pltpu.CompilerParams(
            dimension_semantics=("arbitrary",),
            vmem_limit_bytes=64 * 1024 * 1024,
        ),
    )(x2, row(A_Lambda_re), row(A_Lambda_im), row(A_log_dt), row(A_Dskip), row(gate_w),
      A_B_re, A_B_im, A_C_re, A_C_im, B_w_gate.T, B_w_up.T, B_w_down)
    return out.reshape(Bsz, S, D)


@jax.jit
def pallas_gated_mix__ssm_conv_s5__geglu_ffn__prompt_kernel(
    A_x: jax.Array,
    A_Lambda_re: jax.Array,
    A_Lambda_im: jax.Array,
    A_B_re: jax.Array,
    A_B_im: jax.Array,
    A_C_re: jax.Array,
    A_C_im: jax.Array,
    A_log_dt: jax.Array,
    A_Dskip: jax.Array,
    B_x: jax.Array,
    B_w_gate: jax.Array,
    B_w_up: jax.Array,
    B_w_down: jax.Array,
    gate_w: jax.Array,
):
    return _run(A_x, A_Lambda_re, A_Lambda_im, A_B_re, A_B_im, A_C_re, A_C_im,
                A_log_dt, A_Dskip, B_w_gate, B_w_up, B_w_down, gate_w)
```

```python
import functools

import jax
import jax.numpy as jnp
from jax import lax
import jax.experimental.pallas as pl
import jax.experimental.pallas.tpu as pltpu

F32 = jnp.float32
BF16 = jnp.bfloat16

TM = 256
NSEG = 8


def _cmul(ar, ai, br, bi):
    return ar * br - ai * bi, ar * bi + ai * br


def _kernel(x_ref, lre_ref, lim_ref, ldt_ref, dsk_ref, gw_ref, bre_ref, bim_ref,
            cre_hbm, cim_hbm, wg_hbm, wu_hbm, wd_hbm,
            o_ref,
            lam_ref, wc_ref, z_ref, carry_ref,
            cre_ref, cim_ref, wg_ref, wu_ref, wd_ref, sems, *, tm):
    P = lre_ref.shape[0]
    step = pl.program_id(0)
    nt = (((1,), (1,)), ((), ()))

    copies = [
        pltpu.make_async_copy(wg_hbm, wg_ref, sems.at[0]),
        pltpu.make_async_copy(wu_hbm, wu_ref, sems.at[1]),
        pltpu.make_async_copy(wd_hbm, wd_ref, sems.at[2]),
        pltpu.make_async_copy(cre_hbm, cre_ref, sems.at[3]),
        pltpu.make_async_copy(cim_hbm, cim_ref, sems.at[4]),
    ]

    def ssm_coefs():
        lre = lre_ref[...].astype(F32).reshape(1, P)
        lim = lim_ref[...].astype(F32).reshape(1, P)
        dt = jnp.exp(ldt_ref[...].astype(F32).reshape(1, P)).astype(BF16).astype(F32)
        mag = jnp.exp(dt * lre)
        ang = dt * lim
        lbr = mag * jnp.cos(ang)
        lbi = mag * jnp.sin(ang)
        nr = lbr - 1.0
        ni = lbi
        den = lre * lre + lim * lim
        cr = (nr * lre + ni * lim) / den
        ci = (ni * lre - nr * lim) / den
        return lbr, lbi, cr, ci

    def prep_lam(lbr, lbi):
        pows = [(lbr, lbi)]
        for _ in range(7):
            pows.append(_cmul(pows[-1][0], pows[-1][1], lbr, lbi))
        row = lax.broadcasted_iota(jnp.int32, (8, P), 0)
        for idx, d in enumerate((1, 2, 4)):
            lam_ref[2 * idx] = jnp.where(row >= d, jnp.broadcast_to(pows[d - 1][0], (8, P)), 0.0)
            lam_ref[2 * idx + 1] = jnp.where(row >= d, jnp.broadcast_to(pows[d - 1][1], (8, P)), 0.0)
        lam_ref[6] = jnp.concatenate([p_[0] for p_ in pows], axis=0)
        lam_ref[7] = jnp.concatenate([p_[1] for p_ in pows], axis=0)
        carry_ref[...] = jnp.zeros(carry_ref.shape, F32)

    def prep_wc(cr, ci):
        cre = cre_ref[...].astype(F32)
        cim = cim_ref[...].astype(F32)
        wc_ref[:, 0:P] = (2.0 * (cre * cr - cim * ci)).astype(BF16)
        wc_ref[:, P:2 * P] = (-2.0 * (cre * ci + cim * cr)).astype(BF16)

    def body(first):
        if first:
            for c in copies:
                c.start()
            lbr, lbi, cr, ci = ssm_coefs()
            prep_lam(lbr, lbi)

        x = x_ref[...]
        z_ref[:, 0:P] = lax.dot_general(x, bre_ref[...], nt, preferred_element_type=F32)
        z_ref[:, P:2 * P] = lax.dot_general(x, bim_ref[...], nt, preferred_element_type=F32)

        cr_ = carry_ref[0:1, :]
        ci_ = carry_ref[1:2, :]
        for n in range(tm // 8):
            tr = z_ref[n * 8:(n + 1) * 8, 0:P]
            ti = z_ref[n * 8:(n + 1) * 8, P:2 * P]
            for idx, d in enumerate((1, 2, 4)):
                sr = pltpu.roll(tr, d, 0)
                si = pltpu.roll(ti, d, 0)
                mr, mi = _cmul(lam_ref[2 * idx], lam_ref[2 * idx + 1], sr, si)
                tr = tr + mr
                ti = ti + mi
            mr, mi = _cmul(lam_ref[6], lam_ref[7],
                           jnp.broadcast_to(cr_, (8, P)), jnp.broadcast_to(ci_, (8, P)))
            tr = tr + mr
            ti = ti + mi
            z_ref[n * 8:(n + 1) * 8, 0:P] = tr
            z_ref[n * 8:(n + 1) * 8, P:2 * P] = ti
            cr_ = tr[7:8, :]
            ci_ = ti[7:8, :]
        carry_ref[0:1, :] = cr_
        carry_ref[1:2, :] = ci_

        if first:
            copies[0].wait()
        gate = lax.dot_general(x, wg_ref[...], nt, preferred_element_type=F32)
        if first:
            copies[1].wait()
        up = lax.dot_general(x, wu_ref[...], nt, preferred_element_type=F32)
        act = (jax.nn.gelu(gate, approximate=True) * up).astype(BF16)
        if first:
            copies[2].wait()
        b = jnp.dot(act, wd_ref[...], preferred_element_type=F32)

        if first:
            copies[3].wait()
            copies[4].wait()
            prep_wc(cr, ci)
        xf = x.astype(F32)
        h = z_ref[...].astype(BF16)
        a = lax.dot_general(h, wc_ref[...], nt, preferred_element_type=F32)
        a = a + xf * dsk_ref[...].astype(F32).reshape(1, P)

        logit = jnp.sum(xf * gw_ref[...].astype(F32).reshape(1, P), axis=-1, keepdims=True)
        g = jax.nn.sigmoid(logit)
        o_ref[...] = b + g * (a - b)

    @pl.when(step == 0)
    def _():
        body(True)

    @pl.when(step != 0)
    def _():
        body(False)


@functools.partial(jax.jit, static_argnames=("tm",))
def _run(A_x, A_Lambda_re, A_Lambda_im, A_B_re, A_B_im, A_C_re, A_C_im, A_log_dt,
         A_Dskip, B_w_gate, B_w_up, B_w_down, gate_w, tm=TM):
    Bsz, S, D = A_x.shape
    P = A_Lambda_re.shape[0]
    Fd = B_w_gate.shape[1]
    x2 = A_x.reshape(Bsz * S, D)
    row = lambda v: v.reshape(1, -1)

    full = lambda shape: pl.BlockSpec(shape, lambda i: (0,) * len(shape))
    hbm = pl.BlockSpec(memory_space=pl.ANY)
    out = pl.pallas_call(
        functools.partial(_kernel, tm=tm),
        grid=(S // tm,),
        in_specs=[
            pl.BlockSpec((tm, D), lambda i: (i, 0)),
            full((P,)), full((P,)), full((P,)), full((D,)), full((D,)),
            full((P, D)), full((P, D)),
            hbm, hbm, hbm, hbm, hbm,
        ],
        out_specs=pl.BlockSpec((tm, D), lambda i: (i, 0)),
        out_shape=jax.ShapeDtypeStruct((Bsz * S, D), F32),
        scratch_shapes=[
            pltpu.VMEM((8, 8, P), F32),
            pltpu.VMEM((D, 2 * P), BF16),
            pltpu.VMEM((tm, 2 * P), F32),
            pltpu.VMEM((8, P), F32),
            pltpu.VMEM((D, P), BF16),
            pltpu.VMEM((D, P), BF16),
            pltpu.VMEM((Fd, D), BF16),
            pltpu.VMEM((Fd, D), BF16),
            pltpu.VMEM((Fd, D), BF16),
            pltpu.SemaphoreType.DMA((5,)),
        ],
        compiler_params=pltpu.CompilerParams(
            dimension_semantics=("arbitrary",),
            vmem_limit_bytes=64 * 1024 * 1024,
        ),
    )(x2, A_Lambda_re, A_Lambda_im, A_log_dt, A_Dskip, gate_w,
      A_B_re, A_B_im, A_C_re, A_C_im, B_w_gate.T, B_w_up.T, B_w_down)
    return out.reshape(Bsz, S, D)


@jax.jit
def pallas_gated_mix__ssm_conv_s5__geglu_ffn__prompt_kernel(
    A_x: jax.Array,
    A_Lambda_re: jax.Array,
    A_Lambda_im: jax.Array,
    A_B_re: jax.Array,
    A_B_im: jax.Array,
    A_C_re: jax.Array,
    A_C_im: jax.Array,
    A_log_dt: jax.Array,
    A_Dskip: jax.Array,
    B_x: jax.Array,
    B_w_gate: jax.Array,
    B_w_up: jax.Array,
    B_w_down: jax.Array,
    gate_w: jax.Array,
):
    return _run(A_x, A_Lambda_re, A_Lambda_im, A_B_re, A_B_im, A_C_re, A_C_im,
                A_log_dt, A_Dskip, B_w_gate, B_w_up, B_w_down, gate_w)
```

```python
import functools

import jax
import jax.numpy as jnp
from jax import lax
import jax.experimental.pallas as pl
import jax.experimental.pallas.tpu as pltpu

F32 = jnp.float32
BF16 = jnp.bfloat16

TM = 256
NSEG = 8


def _cmul(ar, ai, br, bi):
    return ar * br - ai * bi, ar * bi + ai * br


def _kernel(xz_ref, xf_ref, lre_ref, lim_ref, ldt_ref, dsk_ref, gw_ref, bre_ref, bim_ref,
            cre_hbm, cim_hbm, wg_hbm, wu_hbm, wd_hbm,
            o_ref,
            lam_ref, wc_ref, z_ref, carry_ref,
            cre_ref, cim_ref, wg_ref, wu_ref, wd_ref, sems, *, tm, nchunk):
    P = lre_ref.shape[0]
    step = pl.program_id(0)
    nt = (((1,), (1,)), ((), ()))

    copies = [
        pltpu.make_async_copy(wg_hbm, wg_ref, sems.at[0]),
        pltpu.make_async_copy(wu_hbm, wu_ref, sems.at[1]),
        pltpu.make_async_copy(wd_hbm, wd_ref, sems.at[2]),
        pltpu.make_async_copy(cre_hbm, cre_ref, sems.at[3]),
        pltpu.make_async_copy(cim_hbm, cim_ref, sems.at[4]),
    ]

    def ssm_coefs():
        lre = lre_ref[...].astype(F32).reshape(1, P)
        lim = lim_ref[...].astype(F32).reshape(1, P)
        dt = jnp.exp(ldt_ref[...].astype(F32).reshape(1, P)).astype(BF16).astype(F32)
        mag = jnp.exp(dt * lre)
        ang = dt * lim
        lbr = mag * jnp.cos(ang)
        lbi = mag * jnp.sin(ang)
        nr = lbr - 1.0
        ni = lbi
        den = lre * lre + lim * lim
        cr = (nr * lre + ni * lim) / den
        ci = (ni * lre - nr * lim) / den
        return lbr, lbi, cr, ci

    def prep_lam():
        lbr, lbi, _, _ = ssm_coefs()
        pows = [(lbr, lbi)]
        for _ in range(7):
            pows.append(_cmul(pows[-1][0], pows[-1][1], lbr, lbi))
        row = lax.broadcasted_iota(jnp.int32, (8, P), 0)
        for idx, d in enumerate((1, 2, 4)):
            lam_ref[2 * idx] = jnp.where(row >= d, jnp.broadcast_to(pows[d - 1][0], (8, P)), 0.0)
            lam_ref[2 * idx + 1] = jnp.where(row >= d, jnp.broadcast_to(pows[d - 1][1], (8, P)), 0.0)
        lam_ref[6] = jnp.concatenate([p_[0] for p_ in pows], axis=0)
        lam_ref[7] = jnp.concatenate([p_[1] for p_ in pows], axis=0)
        carry_ref[...] = jnp.zeros(carry_ref.shape, F32)

    def prep_wc():
        _, _, cr, ci = ssm_coefs()
        cre = cre_ref[...].astype(F32)
        cim = cim_ref[...].astype(F32)
        wc_ref[:, 0:P] = (2.0 * (cre * cr - cim * ci)).astype(BF16)
        wc_ref[:, P:2 * P] = (-2.0 * (cre * ci + cim * cr)).astype(BF16)

    def stage_a(zb_ref):
        x = xz_ref[...]
        zb_ref[:, 0:P] = lax.dot_general(x, bre_ref[...], nt, preferred_element_type=F32)
        zb_ref[:, P:2 * P] = lax.dot_general(x, bim_ref[...], nt, preferred_element_type=F32)
        cr_ = carry_ref[0:1, :]
        ci_ = carry_ref[1:2, :]
        for n in range(tm // 8):
            tr = zb_ref[n * 8:(n + 1) * 8, 0:P]
            ti = zb_ref[n * 8:(n + 1) * 8, P:2 * P]
            for idx, d in enumerate((1, 2, 4)):
                sr = pltpu.roll(tr, d, 0)
                si = pltpu.roll(ti, d, 0)
                mr, mi = _cmul(lam_ref[2 * idx], lam_ref[2 * idx + 1], sr, si)
                tr = tr + mr
                ti = ti + mi
            mr, mi = _cmul(lam_ref[6], lam_ref[7],
                           jnp.broadcast_to(cr_, (8, P)), jnp.broadcast_to(ci_, (8, P)))
            tr = tr + mr
            ti = ti + mi
            zb_ref[n * 8:(n + 1) * 8, 0:P] = tr
            zb_ref[n * 8:(n + 1) * 8, P:2 * P] = ti
            cr_ = tr[7:8, :]
            ci_ = ti[7:8, :]
        carry_ref[0:1, :] = cr_
        carry_ref[1:2, :] = ci_

    def stage_b(hb_ref, first):
        x = xf_ref[...]
        if first:
            copies[0].wait()
        gate = lax.dot_general(x, wg_ref[...], nt, preferred_element_type=F32)
        if first:
            copies[1].wait()
        up = lax.dot_general(x, wu_ref[...], nt, preferred_element_type=F32)
        act = (jax.nn.gelu(gate, approximate=True) * up).astype(BF16)
        if first:
            copies[2].wait()
        b = jnp.dot(act, wd_ref[...], preferred_element_type=F32)
        if first:
            copies[3].wait()
            copies[4].wait()
            prep_wc()
        xf = x.astype(F32)
        h = hb_ref[...].astype(BF16)
        a = lax.dot_general(h, wc_ref[...], nt, preferred_element_type=F32)
        a = a + xf * dsk_ref[...].astype(F32).reshape(1, P)
        logit = jnp.sum(xf * gw_ref[...].astype(F32).reshape(1, P), axis=-1, keepdims=True)
        g = jax.nn.sigmoid(logit)
        o_ref[...] = b + g * (a - b)

    @pl.when(step == 0)
    def _():
        for c in copies:
            c.start()
        prep_lam()
        stage_a(z_ref.at[0])

    @pl.when(step == 1)
    def _():
        stage_b(z_ref.at[0], True)
        stage_a(z_ref.at[1])

    for parity in (0, 1):
        @pl.when(jnp.logical_and(jnp.logical_and(step > 1, step < nchunk), step % 2 == parity))
        def _():
            stage_b(z_ref.at[1 - parity], False)
            stage_a(z_ref.at[parity])

    @pl.when(step == nchunk)
    def _():
        stage_b(z_ref.at[(nchunk - 1) % 2], False)


@functools.partial(jax.jit, static_argnames=("tm",))
def _run(A_x, A_Lambda_re, A_Lambda_im, A_B_re, A_B_im, A_C_re, A_C_im, A_log_dt,
         A_Dskip, B_w_gate, B_w_up, B_w_down, gate_w, tm=TM):
    Bsz, S, D = A_x.shape
    P = A_Lambda_re.shape[0]
    Fd = B_w_gate.shape[1]
    x2 = A_x.reshape(Bsz * S, D)
    nchunk = S // tm

    full = lambda shape: pl.BlockSpec(shape, lambda i: (0,) * len(shape))
    hbm = pl.BlockSpec(memory_space=pl.ANY)
    out = pl.pallas_call(
        functools.partial(_kernel, tm=tm, nchunk=nchunk),
        grid=(nchunk + 1,),
        in_specs=[
            pl.BlockSpec((tm, D), lambda i: (jnp.minimum(i, nchunk - 1), 0)),
            pl.BlockSpec((tm, D), lambda i: (jnp.maximum(i - 1, 0), 0)),
            full((P,)), full((P,)), full((P,)), full((D,)), full((D,)),
            full((P, D)), full((P, D)),
            hbm, hbm, hbm, hbm, hbm,
        ],
        out_specs=pl.BlockSpec((tm, D), lambda i: (jnp.maximum(i - 1, 0), 0)),
        out_shape=jax.ShapeDtypeStruct((Bsz * S, D), F32),
        scratch_shapes=[
            pltpu.VMEM((8, 8, P), F32),
            pltpu.VMEM((D, 2 * P), BF16),
            pltpu.VMEM((2, tm, 2 * P), F32),
            pltpu.VMEM((8, P), F32),
            pltpu.VMEM((D, P), BF16),
            pltpu.VMEM((D, P), BF16),
            pltpu.VMEM((Fd, D), BF16),
            pltpu.VMEM((Fd, D), BF16),
            pltpu.VMEM((Fd, D), BF16),
            pltpu.SemaphoreType.DMA((5,)),
        ],
        compiler_params=pltpu.CompilerParams(
            dimension_semantics=("arbitrary",),
            vmem_limit_bytes=64 * 1024 * 1024,
        ),
    )(x2, x2, A_Lambda_re, A_Lambda_im, A_log_dt, A_Dskip, gate_w,
      A_B_re, A_B_im, A_C_re, A_C_im, B_w_gate.T, B_w_up.T, B_w_down)
    return out.reshape(Bsz, S, D)


@jax.jit
def pallas_gated_mix__ssm_conv_s5__geglu_ffn__prompt_kernel(
    A_x: jax.Array,
    A_Lambda_re: jax.Array,
    A_Lambda_im: jax.Array,
    A_B_re: jax.Array,
    A_B_im: jax.Array,
    A_C_re: jax.Array,
    A_C_im: jax.Array,
    A_log_dt: jax.Array,
    A_Dskip: jax.Array,
    B_x: jax.Array,
    B_w_gate: jax.Array,
    B_w_up: jax.Array,
    B_w_down: jax.Array,
    gate_w: jax.Array,
):
    return _run(A_x, A_Lambda_re, A_Lambda_im, A_B_re, A_B_im, A_C_re, A_C_im,
                A_log_dt, A_Dskip, B_w_gate, B_w_up, B_w_down, gate_w)
```

```python
import functools

import jax
import jax.numpy as jnp
from jax import lax
import jax.experimental.pallas as pl
import jax.experimental.pallas.tpu as pltpu

F32 = jnp.float32
BF16 = jnp.bfloat16

TM = 256
NSEG = 8


def _cmul(ar, ai, br, bi):
    return ar * br - ai * bi, ar * bi + ai * br


def _kernel(x_ref, lre_ref, lim_ref, ldt_ref, dsk_ref, gw_ref, bre_ref, bim_ref,
            cre_hbm, cim_hbm, wg_hbm, wu_hbm, wd_hbm,
            o_ref,
            lam_ref, wc_ref, z_ref, carry_ref,
            cre_ref, cim_ref, wg_ref, wu_ref, wd_ref, sems, *, tm):
    P = lre_ref.shape[0]
    step = pl.program_id(0)
    nt = (((1,), (1,)), ((), ()))

    copies = [
        pltpu.make_async_copy(wg_hbm, wg_ref, sems.at[0]),
        pltpu.make_async_copy(wu_hbm, wu_ref, sems.at[1]),
        pltpu.make_async_copy(wd_hbm, wd_ref, sems.at[2]),
        pltpu.make_async_copy(cre_hbm, cre_ref, sems.at[3]),
        pltpu.make_async_copy(cim_hbm, cim_ref, sems.at[4]),
    ]

    def ssm_coefs():
        lre = lre_ref[...].astype(F32).reshape(1, P)
        lim = lim_ref[...].astype(F32).reshape(1, P)
        dt = jnp.exp(ldt_ref[...].astype(F32).reshape(1, P)).astype(BF16).astype(F32)
        mag = jnp.exp(dt * lre)
        ang = dt * lim
        lbr = mag * jnp.cos(ang)
        lbi = mag * jnp.sin(ang)
        nr = lbr - 1.0
        ni = lbi
        den = lre * lre + lim * lim
        cr = (nr * lre + ni * lim) / den
        ci = (ni * lre - nr * lim) / den
        return lbr, lbi, cr, ci

    def prep_lam(lbr, lbi):
        pows = [(lbr, lbi)]
        for _ in range(7):
            pows.append(_cmul(pows[-1][0], pows[-1][1], lbr, lbi))
        row = lax.broadcasted_iota(jnp.int32, (8, P), 0)
        for idx, d in enumerate((1, 2, 4)):
            lam_ref[2 * idx] = jnp.where(row >= d, jnp.broadcast_to(pows[d - 1][0], (8, P)), 0.0)
            lam_ref[2 * idx + 1] = jnp.where(row >= d, jnp.broadcast_to(pows[d - 1][1], (8, P)), 0.0)
        lam_ref[6] = jnp.concatenate([p_[0] for p_ in pows], axis=0)
        lam_ref[7] = jnp.concatenate([p_[1] for p_ in pows], axis=0)
        carry_ref[...] = jnp.zeros(carry_ref.shape, F32)

    def prep_wc(cr, ci):
        cre = cre_ref[...].astype(F32)
        cim = cim_ref[...].astype(F32)
        wc_ref[:, 0:P] = (2.0 * (cre * cr - cim * ci)).astype(BF16)
        wc_ref[:, P:2 * P] = (-2.0 * (cre * ci + cim * cr)).astype(BF16)

    def body(first):
        if first:
            copies[0].start()
            copies[1].start()
            lbr, lbi, cr, ci = ssm_coefs()
            prep_lam(lbr, lbi)

        x = x_ref[...]
        z_ref[:, 0:P] = lax.dot_general(x, bre_ref[...], nt, preferred_element_type=F32)
        z_ref[:, P:2 * P] = lax.dot_general(x, bim_ref[...], nt, preferred_element_type=F32)

        cr_ = carry_ref[0:1, :]
        ci_ = carry_ref[1:2, :]
        for n in range(tm // 8):
            tr = z_ref[n * 8:(n + 1) * 8, 0:P]
            ti = z_ref[n * 8:(n + 1) * 8, P:2 * P]
            for idx, d in enumerate((1, 2, 4)):
                sr = pltpu.roll(tr, d, 0)
                si = pltpu.roll(ti, d, 0)
                mr, mi = _cmul(lam_ref[2 * idx], lam_ref[2 * idx + 1], sr, si)
                tr = tr + mr
                ti = ti + mi
            mr, mi = _cmul(lam_ref[6], lam_ref[7],
                           jnp.broadcast_to(cr_, (8, P)), jnp.broadcast_to(ci_, (8, P)))
            tr = tr + mr
            ti = ti + mi
            z_ref[n * 8:(n + 1) * 8, 0:P] = tr
            z_ref[n * 8:(n + 1) * 8, P:2 * P] = ti
            cr_ = tr[7:8, :]
            ci_ = ti[7:8, :]
        carry_ref[0:1, :] = cr_
        carry_ref[1:2, :] = ci_

        if first:
            copies[0].wait()
            copies[2].start()
        gate = lax.dot_general(x, wg_ref[...], nt, preferred_element_type=F32)
        if first:
            copies[1].wait()
            copies[3].start()
            copies[4].start()
        up = lax.dot_general(x, wu_ref[...], nt, preferred_element_type=F32)
        act = (jax.nn.gelu(gate, approximate=True) * up).astype(BF16)
        if first:
            copies[2].wait()
        b = jnp.dot(act, wd_ref[...], preferred_element_type=F32)

        if first:
            copies[3].wait()
            copies[4].wait()
            prep_wc(cr, ci)
        xf = x.astype(F32)
        h = z_ref[...].astype(BF16)
        a = lax.dot_general(h, wc_ref[...], nt, preferred_element_type=F32)
        a = a + xf * dsk_ref[...].astype(F32).reshape(1, P)

        logit = jnp.sum(xf * gw_ref[...].astype(F32).reshape(1, P), axis=-1, keepdims=True)
        g = jax.nn.sigmoid(logit)
        o_ref[...] = b + g * (a - b)

    @pl.when(step == 0)
    def _():
        body(True)

    @pl.when(step != 0)
    def _():
        body(False)


@functools.partial(jax.jit, static_argnames=("tm",))
def _run(A_x, A_Lambda_re, A_Lambda_im, A_B_re, A_B_im, A_C_re, A_C_im, A_log_dt,
         A_Dskip, B_w_gate, B_w_up, B_w_down, gate_w, tm=TM):
    Bsz, S, D = A_x.shape
    P = A_Lambda_re.shape[0]
    Fd = B_w_gate.shape[1]
    x2 = A_x.reshape(Bsz * S, D)
    row = lambda v: v.reshape(1, -1)

    full = lambda shape: pl.BlockSpec(shape, lambda i: (0,) * len(shape))
    hbm = pl.BlockSpec(memory_space=pl.ANY)
    out = pl.pallas_call(
        functools.partial(_kernel, tm=tm),
        grid=(S // tm,),
        in_specs=[
            pl.BlockSpec((tm, D), lambda i: (i, 0)),
            full((P,)), full((P,)), full((P,)), full((D,)), full((D,)),
            full((P, D)), full((P, D)),
            hbm, hbm, hbm, hbm, hbm,
        ],
        out_specs=pl.BlockSpec((tm, D), lambda i: (i, 0)),
        out_shape=jax.ShapeDtypeStruct((Bsz * S, D), F32),
        scratch_shapes=[
            pltpu.VMEM((8, 8, P), F32),
            pltpu.VMEM((D, 2 * P), BF16),
            pltpu.VMEM((tm, 2 * P), F32),
            pltpu.VMEM((8, P), F32),
            pltpu.VMEM((D, P), BF16),
            pltpu.VMEM((D, P), BF16),
            pltpu.VMEM((Fd, D), BF16),
            pltpu.VMEM((Fd, D), BF16),
            pltpu.VMEM((Fd, D), BF16),
            pltpu.SemaphoreType.DMA((5,)),
        ],
        compiler_params=pltpu.CompilerParams(
            dimension_semantics=("arbitrary",),
            vmem_limit_bytes=64 * 1024 * 1024,
        ),
    )(x2, A_Lambda_re, A_Lambda_im, A_log_dt, A_Dskip, gate_w,
      A_B_re, A_B_im, A_C_re, A_C_im, B_w_gate.T, B_w_up.T, B_w_down)
    return out.reshape(Bsz, S, D)


@jax.jit
def pallas_gated_mix__ssm_conv_s5__geglu_ffn__prompt_kernel(
    A_x: jax.Array,
    A_Lambda_re: jax.Array,
    A_Lambda_im: jax.Array,
    A_B_re: jax.Array,
    A_B_im: jax.Array,
    A_C_re: jax.Array,
    A_C_im: jax.Array,
    A_log_dt: jax.Array,
    A_Dskip: jax.Array,
    B_x: jax.Array,
    B_w_gate: jax.Array,
    B_w_up: jax.Array,
    B_w_down: jax.Array,
    gate_w: jax.Array,
):
    return _run(A_x, A_Lambda_re, A_Lambda_im, A_B_re, A_B_im, A_C_re, A_C_im,
                A_log_dt, A_Dskip, B_w_gate, B_w_up, B_w_down, gate_w)
```
